```python
import os as _os
_os.environ.setdefault('JAX_PLATFORMS', 'cpu')
import jax
import jax.numpy as jnp

def _softmax(x, axis=-1):
    return jax.nn.softmax(x, axis=axis)

def _gelu(x):
    return jax.nn.gelu(x, approximate=True)

def _silu(x):
    return jax.nn.silu(x)

def _sigmoid(x):
    return jax.nn.sigmoid(x)

def _layernorm(x, axis=-1, eps=1e-05):
    m = jnp.mean(x, axis=axis, keepdims=True)
    v = jnp.var(x, axis=axis, keepdims=True)
    return (x - m) / jnp.sqrt(v + eps)

def _scatter_add(tgt, idx, src, axis=0):
    return tgt.at[idx].add(src)

def _segment_sum(src, seg, n):
    return jax.ops.segment_sum(src, seg, n)

class _Rng:

    def __init__(self, key):
        self._k = key

    def _next(self):
        self._k, sub = jax.random.split(self._k)
        return sub

    def normal(self, shape):
        return jax.random.normal(self._next(), shape, dtype=jnp.bfloat16)

    def randint(self, lo, hi, shape):
        return jax.random.randint(self._next(), shape, lo, hi, dtype=jnp.int32)

    def uniform(self, shape, lo=0.0, hi=1.0):
        return jax.random.uniform(self._next(), shape, jnp.bfloat16, lo, hi)

    def permutation(self, n):
        return jax.random.permutation(self._next(), n)
kernel_name = 'adaLN_cond__mha_block__geglu_ffn__prompt'

def setup_inputs():
    _rng = _Rng(jax.random.key(int.from_bytes(__import__("os").urandom(4), "little")))
    _w = lambda a: (lambda t: t.astype(jnp.bfloat16) if jnp.issubdtype(t.dtype, jnp.floating) else t)(jnp.asarray(a))

    def _A_setup():
        B, S, D, H = (1, 2048, 640, 32)
        return {'x': _w((lambda *s: _rng.normal(s) * 0.05)(B, S, D)), 'wqkv': _w((lambda *s: _rng.normal(s) * 0.05)(D, 3 * D)), 'wo': _w((lambda *s: _rng.normal(s) * 0.05)(D, D))}
    _A_in = _A_setup()

    def _B_setup():
        B, S, D, F = (1, 2048, 640, 1728)
        return {'x': _w((lambda *s: _rng.normal(s) * 0.05)(B, S, D)), 'w_gate': _w((lambda *s: _rng.normal(s) * 0.05)(D, F)), 'w_up': _w((lambda *s: _rng.normal(s) * 0.05)(D, F)), 'w_down': _w((lambda *s: _rng.normal(s) * 0.05)(F, D))}
    _B_in = _B_setup()
    return {'A_x': _A_in['x'], 'A_wqkv': _A_in['wqkv'], 'A_wo': _A_in['wo'], 'B_x': _B_in['x'], 'B_w_gate': _B_in['w_gate'], 'B_w_up': _B_in['w_up'], 'B_w_down': _B_in['w_down'], 'c': _w((lambda *s: _rng.normal(s) * 0.05)(1, 640) * 8.0), 'w_mod': _w((lambda *s: _rng.normal(s) * 0.05)(640, 6 * 640) * 640 ** (-0.5) * 8.0)}

def reference(A_x, A_wqkv, A_wo, B_x, B_w_gate, B_w_up, B_w_down, c, w_mod):

    def _A_ref(x, wqkv, wo):
        B, S, D = x.shape
        H = 32
        Dh = D // H
        qkv = (lambda x, *d: x.transpose(*d))((x @ wqkv).reshape(B, S, 3, H, Dh), 2, 0, 3, 1, 4)
        q, k, v = (qkv[0], qkv[1], qkv[2])
        scores = jnp.einsum('bhqd,bhkd->bhqk', q, k) * Dh ** (-0.5)
        p = _softmax(scores, axis=-1)
        o = jnp.einsum('bhqk,bhkd->bhqd', p, v)
        return (lambda x, *d: x.transpose(*d))(o, 0, 2, 1, 3).reshape(B, S, D) @ wo

    def _B_ref(x, w_gate, w_up, w_down):
        return _gelu(x @ w_gate) * (x @ w_up) @ w_down
    x = A_x
    mod = (_silu(c) @ w_mod).reshape(c.shape[0], 6, 1, -1)
    sa, ca, ga, sb, cb, gb = (mod[:, 0].copy(), mod[:, 1].copy(), mod[:, 2].copy(), mod[:, 3].copy(), mod[:, 4].copy(), mod[:, 5].copy())
    h = _layernorm(x, axis=-1) * (1 + ca) + sa
    x = x + ga * _A_ref(h, A_wqkv, A_wo)
    h = _layernorm(x, axis=-1) * (1 + cb) + sb
    x = x + gb * _B_ref(h, B_w_gate, B_w_up, B_w_down)
    return x
```

```python
import functools
import math

import jax
import jax.numpy as jnp
from jax.experimental import pallas as pl
from jax.experimental.pallas import tpu as pltpu

S = 2048
D = 640
H = 32
DH = 20
F = 1728
TQ = 512
NQ = S // TQ
CK = 128
NC = S // CK
NA = 12
UN = 4
NW = 6
VR = 24
EPS = 1e-5
FC = 256

_NT = (((1,), (1,)), ((), ()))
_TN = (((0,), (0,)), ((), ()))
_F32 = jnp.float32
_BF16 = jnp.bfloat16


def _win_start(g):
    return 120 * g if g < NW - 1 else D - 128


def _layernorm(xf):
    m = jnp.mean(xf, axis=-1, keepdims=True)
    xc = xf - m
    v = jnp.mean(xc * xc, axis=-1, keepdims=True)
    return xc * jax.lax.rsqrt(v + EPS)


def _gelu_tanh(x):
    c = math.sqrt(2.0 / math.pi)
    return 0.5 * x * (1.0 + jnp.tanh(c * (x + 0.044715 * (x * x * x))))


def _dot(a, b):
    return jnp.dot(a, b, preferred_element_type=_F32)


def _dot_nt(a, b):
    return jax.lax.dot_general(a, b, _NT, preferred_element_type=_F32)


def _dot_tn(a, b):
    return jax.lax.dot_general(a, b, _TN, preferred_element_type=_F32)


def _kernel(c_ref, x_hbm, wqkv_hbm, wo_hbm, wg_hbm, wu_hbm, wd_hbm, wmod_hbm,
            o_hbm,
            x_v, wq_v, wk_v, wv_v, wo_v, wg_v, wu_v, wd_v, wmoda_v, wmodb_v,
            mod_s, h_s, wqw_s, wkw_s, wvt_s, kw_s, q_s, vt_s, s1, ot_s, o_v,
            sems, xsems, osems):
    cp_wk = pltpu.make_async_copy(wqkv_hbm.at[:, D:2 * D], wk_v, sems.at[0])
    cp_ma = pltpu.make_async_copy(wmod_hbm.at[:, 0:2 * D], wmoda_v, sems.at[1])
    cp_wq = pltpu.make_async_copy(wqkv_hbm.at[:, 0:D], wq_v, sems.at[2])
    cp_wv = pltpu.make_async_copy(wqkv_hbm.at[:, 2 * D:3 * D], wv_v, sems.at[3])
    cp_wo = pltpu.make_async_copy(wo_hbm, wo_v, sems.at[4])
    cp_mb = pltpu.make_async_copy(wmod_hbm.at[:, 2 * D:6 * D], wmodb_v, sems.at[5])
    cp_wg = pltpu.make_async_copy(wg_hbm, wg_v, sems.at[6])
    cp_wu = pltpu.make_async_copy(wu_hbm, wu_v, sems.at[7])
    cp_wd = pltpu.make_async_copy(wd_hbm, wd_v, sems.at[8])

    lane = jax.lax.broadcasted_iota(jnp.int32, (TQ, 128), 1)

    def get_qm(qt, h):
        g = (h * 43) >> 8
        off = DH * h - 120 * g + jnp.where(g == NW - 1, 120 * (NW - 1) - (D - 128), 0)
        qw = q_s[g, pl.ds(pl.multiple_of(qt * TQ, TQ), TQ), :]
        mask = (lane >= off) & (lane < off + DH)
        return g, jnp.where(mask, qw, jnp.zeros_like(qw))

    def qk(g, qm, c):
        return _dot_nt(kw_s[g, c * CK:(c + 1) * CK, :], qm)

    def stage1_store(s, c, mx):
        s1[c * CK:(c + 1) * CK, :] = s
        cm = jnp.max(s.reshape(CK // 8, 8, TQ), axis=0)
        return cm if mx is None else jnp.maximum(mx, cm)

    qscale = (DH ** -0.5) * math.log2(math.e)

    def rows_of(r):
        if isinstance(r, int):
            return slice(r * TQ, (r + 1) * TQ)
        return pl.ds(pl.multiple_of(r * TQ, TQ), TQ)

    def ln1(r):
        rows = rows_of(r)
        xf = x_v[rows, :].astype(_F32)
        h_s[rows, :] = (_layernorm(xf) * (1.0 + mod_s[0:1, D:2 * D]) + mod_s[0:1, 0:D]).astype(_BF16)

    def kproj(r):
        rows = rows_of(r)
        kk = _dot(h_s[rows, :], wkw_s[...]).astype(_BF16)
        for g in range(NW):
            kw_s[g, rows, :] = kk[:, 128 * g:128 * (g + 1)]

    def qproj(r):
        rows = rows_of(r)
        qq = (_dot(h_s[rows, :], wqw_s[...]) * qscale).astype(_BF16)
        for g in range(NW):
            q_s[g, rows, :] = qq[:, 128 * g:128 * (g + 1)]

    def vproj(r):
        rows = rows_of(r)
        vt = _dot_nt(wvt_s[...], h_s[rows, :])
        tail = jnp.where(jax.lax.broadcasted_iota(jnp.int32, (VR - DH, TQ), 0) == 0, 1.0, 0.0)
        for h in range(H):
            vt_s[h, 0:DH, rows] = vt[DH * h:DH * (h + 1), :]
            vt_s[h, DH:VR, rows] = tail

    def x_copy(r):
        rows = rows_of(r)
        return pltpu.make_async_copy(x_hbm.at[rows, :], x_v.at[rows, :], xsems.at[r])

    with jax.named_scope('prologue'):
        cp_wk.start()
        cp_ma.start()
        x_copy(0).start()

        cp_wk.wait()
        x_copy(1).start()
        cp_wq.start()
        for g in range(NW):
            c0 = _win_start(g)
            wkw_s[:, 128 * g:128 * (g + 1)] = wk_v[:, c0:c0 + 128]
        cf = c_ref[...].astype(_F32)
        sc = jnp.broadcast_to(cf * jax.nn.sigmoid(cf), (8, D))
        cp_ma.wait()
        x_copy(2).start()
        x_copy(3).start()
        cp_wv.start()
        mod_s[:, 0:2 * D] = _dot(sc, wmoda_v[...])
        x_copy(0).wait()
        cp_mb.start()
        cp_wo.start()
        cp_wg.start()
        cp_wu.start()
        cp_wd.start()
        ln1(0)

        def kloop(r, _):
            @pl.when(r < NQ - 1)
            def _():
                x_copy(r + 1).wait()
            kproj(r)
            ln1(jnp.minimum(r + 1, NQ - 1))
            return 0
        jax.lax.fori_loop(0, NQ, kloop, 0)

        cp_wq.wait()
        cp_wv.wait()
        cp_mb.wait()
        mod_s[:, 2 * D:6 * D] = _dot(sc, wmodb_v[...])
        for g in range(NW):
            c0 = _win_start(g)
            wqw_s[:, 128 * g:128 * (g + 1)] = wq_v[:, c0:c0 + 128]
        wvt_s[...] = wv_v[...].astype(_F32).T

        def qvloop(r, _):
            qproj(r)
            vproj(r)
            return 0
        jax.lax.fori_loop(0, NQ, qvloop, 0)

        g0, qm0 = get_qm(0, 0)
        mx = None
        for c in range(NC):
            mx = stage1_store(qk(g0, qm0, c), c, mx)
            if c == NA - 1:
                ma0 = jnp.max(mx, axis=0, keepdims=True)
        mb0 = jnp.max(mx, axis=0, keepdims=True)
        cp_wo.wait()
        cp_wg.wait()
        cp_wu.wait()
        cp_wd.wait()

    def out_copy(i):
        return pltpu.make_async_copy(
            o_v.at[i % 2], o_hbm.at[pl.ds(pl.multiple_of(i * TQ, TQ), TQ), :], osems.at[i % 2])

    def tile(i, ms):
        def unit(b, k, ms):
            ma, mb = ms
            h = b * UN + k
            hn = (h + 1) & (H - 1)
            qtn = jnp.minimum(i + ((h + 1) >> 5), NQ - 1)
            g, qm = get_qm(qtn, hn)
            mx = None
            acc = None
            for c in range(NC):
                if c == NA:
                    acc = acc * jnp.exp2(ma - mb)
                p = jnp.exp2(s1[c * CK:(c + 1) * CK, :] - (ma if c < NA else mb)).astype(_BF16)
                s = qk(g, qm, c)
                o = _dot(vt_s[h, :, c * CK:(c + 1) * CK], p)
                acc = o if acc is None else acc + o
                mx = stage1_store(s, c, mx)
                if c == NA - 1:
                    ma_n = jnp.max(mx, axis=0, keepdims=True)
            on = acc * (1.0 / acc[DH:DH + 1, :])
            ot_s[b, DH * k:DH * (k + 1), :] = on[0:DH, :]
            return ma_n, jnp.max(mx, axis=0, keepdims=True)

        def body(b, ms):
            for k in range(UN):
                ms = unit(b, k, ms)
            return ms

        with jax.named_scope('attn'):
            ms = jax.lax.fori_loop(0, H // UN, body, ms)

        sa, ca, ga, sb, cb, gb = [mod_s[0:1, k * D:(k + 1) * D] for k in range(6)]
        with jax.named_scope('post'):
            HB = TQ // 2
            x1, h2 = [], []
            for a in range(2):
                ot = ot_s[:, :, a * HB:(a + 1) * HB].reshape(D, HB)
                attn = _dot_tn(ot, wo_v[...])
                xt = x_v[pl.ds(pl.multiple_of(i * TQ + a * HB, HB), HB), :].astype(_F32)
                x1.append(xt + ga * attn)
            for a in range(2):
                h2.append((_layernorm(x1[a]) * (1.0 + cb) + sb).astype(_BF16))
            acts = []
            for a in range(2):
                gt = _dot_nt(h2[a], wg_v[0:FC, :])
                up = _dot_nt(h2[a], wu_v[0:FC, :])
                acts.append((_gelu_tanh(gt) * up).astype(_BF16))
            act = jnp.concatenate(acts, axis=0)
            h2 = jnp.concatenate(h2, axis=0)
            y = _dot(act, wd_v[0:FC, :])
            for f0 in range(FC, F, FC):
                f1 = min(f0 + FC, F)
                gt = _dot_nt(h2, wg_v[f0:f1, :])
                up = _dot_nt(h2, wu_v[f0:f1, :])
                act = (_gelu_tanh(gt) * up).astype(_BF16)
                y = y + _dot(act, wd_v[f0:f1, :])
            x1 = jnp.concatenate(x1, axis=0)

            @pl.when(i >= 2)
            def _():
                out_copy(i - 2).wait()
            o_v[i % 2] = (x1 + gb * y).astype(o_v.dtype)
            out_copy(i).start()
        return ms

    jax.lax.fori_loop(0, NQ, tile, (ma0, mb0))
    out_copy(NQ - 2).wait()
    out_copy(NQ - 1).wait()


@jax.jit
def pallas_adaLN_cond__mha_block__geglu_ffn__prompt_kernel(
    A_x, A_wqkv, A_wo, B_x, B_w_gate, B_w_up, B_w_down, c, w_mod,
):
    del B_x
    x2 = A_x.reshape(S, D)
    hbm = pl.BlockSpec(memory_space=pltpu.MemorySpace.HBM)
    out = pl.pallas_call(
        _kernel,
        in_specs=[pl.BlockSpec(memory_space=pltpu.MemorySpace.VMEM)] + [hbm] * 7,
        out_specs=hbm,
        out_shape=jax.ShapeDtypeStruct((S, D), A_x.dtype),
        scratch_shapes=[
            pltpu.VMEM((S, D), _BF16),
            pltpu.VMEM((D, D), _BF16),
            pltpu.VMEM((D, D), _BF16),
            pltpu.VMEM((D, D), _BF16),
            pltpu.VMEM((D, D), _BF16),
            pltpu.VMEM((F, D), _BF16),
            pltpu.VMEM((F, D), _BF16),
            pltpu.VMEM((F, D), _BF16),
            pltpu.VMEM((D, 2 * D), _BF16),
            pltpu.VMEM((D, 4 * D), _BF16),
            pltpu.VMEM((8, 6 * D), _F32),
            pltpu.VMEM((S, D), _BF16),
            pltpu.VMEM((D, NW * 128), _BF16),
            pltpu.VMEM((D, NW * 128), _BF16),
            pltpu.VMEM((D, D), _F32),
            pltpu.VMEM((NW, S, 128), _BF16),
            pltpu.VMEM((NW, S, 128), _BF16),
            pltpu.VMEM((H, VR, S), _F32),
            pltpu.VMEM((S, TQ), _F32),
            pltpu.VMEM((H // UN, UN * DH, TQ), _F32),
            pltpu.VMEM((2, TQ, D), _BF16),
            pltpu.SemaphoreType.DMA((9,)),
            pltpu.SemaphoreType.DMA((NQ,)),
            pltpu.SemaphoreType.DMA((2,)),
        ],
        compiler_params=pltpu.CompilerParams(
            vmem_limit_bytes=100 * 1024 * 1024,
        ),
    )(c, x2, A_wqkv, A_wo, B_w_gate.T, B_w_up.T, B_w_down, w_mod)
    return out.reshape(A_x.shape)
```

```python
import functools
import math

import jax
import jax.numpy as jnp
from jax.experimental import pallas as pl
from jax.experimental.pallas import tpu as pltpu

S = 2048
D = 640
H = 32
DH = 20
F = 1728
TQ = 512
NQ = S // TQ
CK = 128
NC = S // CK
NA = 12
UN = 8
NW = 6
VR = 24
EPS = 1e-5
FC = 256

_NT = (((1,), (1,)), ((), ()))
_TN = (((0,), (0,)), ((), ()))
_F32 = jnp.float32
_BF16 = jnp.bfloat16


def _win_start(g):
    return 120 * g if g < NW - 1 else D - 128


def _layernorm(xf):
    m = jnp.mean(xf, axis=-1, keepdims=True)
    xc = xf - m
    v = jnp.mean(xc * xc, axis=-1, keepdims=True)
    return xc * jax.lax.rsqrt(v + EPS)


def _gelu_tanh(x):
    c = math.sqrt(2.0 / math.pi)
    return 0.5 * x * (1.0 + jnp.tanh(c * (x + 0.044715 * (x * x * x))))


def _dot(a, b):
    return jnp.dot(a, b, preferred_element_type=_F32)


def _dot_nt(a, b):
    return jax.lax.dot_general(a, b, _NT, preferred_element_type=_F32)


def _dot_tn(a, b):
    return jax.lax.dot_general(a, b, _TN, preferred_element_type=_F32)


def _kernel(c_ref, x_hbm, wqkv_hbm, wo_hbm, wg_hbm, wu_hbm, wd_hbm, wmod_hbm,
            o_hbm,
            s1, kq_s, vt_s, ot_s,
            x_v, wq_v, wk_v, wv_v, wo_v, wg_v, wu_v, wd_v, wmoda_v, wmodb_v,
            mod_s, modb_s, h_s, o_v,
            sems, xsems, osems):
    cp_wk = pltpu.make_async_copy(wqkv_hbm.at[:, D:2 * D], wk_v, sems.at[0])
    cp_ma = pltpu.make_async_copy(wmod_hbm.at[:, 0:2 * D], wmoda_v, sems.at[1])
    cp_wq = pltpu.make_async_copy(wqkv_hbm.at[:, 0:D], wq_v, sems.at[2])
    cp_wv = pltpu.make_async_copy(wqkv_hbm.at[:, 2 * D:3 * D], wv_v, sems.at[3])
    cp_wo = pltpu.make_async_copy(wo_hbm, wo_v, sems.at[4])
    cp_mb = pltpu.make_async_copy(wmod_hbm.at[:, 2 * D:6 * D], wmodb_v, sems.at[5])
    cp_wg = pltpu.make_async_copy(wg_hbm, wg_v, sems.at[6])
    cp_wu = pltpu.make_async_copy(wu_hbm, wu_v, sems.at[7])
    cp_wd = pltpu.make_async_copy(wd_hbm, wd_v, sems.at[8])

    lane = jax.lax.broadcasted_iota(jnp.int32, (TQ, 128), 1)

    def get_qm(qt, h):
        g = (h * 43) >> 8
        off = DH * h - 120 * g + jnp.where(g == NW - 1, 120 * (NW - 1) - (D - 128), 0)
        qw = kq_s[1, g, pl.ds(pl.multiple_of(qt * TQ, TQ), TQ), :]
        mask = (lane >= off) & (lane < off + DH)
        return g, jnp.where(mask, qw, jnp.zeros_like(qw))

    def qk(g, qm, c):
        return _dot_nt(kq_s[0, g, c * CK:(c + 1) * CK, :], qm)

    def stage1_store(s, c, mx):
        s1[c * CK:(c + 1) * CK, :] = s
        cm = jnp.max(s.reshape(CK // 8, 8, TQ), axis=0)
        return cm if mx is None else jnp.maximum(mx, cm)

    qscale = (DH ** -0.5) * math.log2(math.e)

    def rows_of(r):
        if isinstance(r, int):
            return slice(r * TQ, (r + 1) * TQ)
        return pl.ds(pl.multiple_of(r * TQ, TQ), TQ)

    RB = 128

    def ln1(r, blk=None):
        if blk is None:
            rows = rows_of(r)
        else:
            rows = pl.ds(pl.multiple_of(r * TQ + blk * RB, RB), RB)
        xf = x_v[rows, :].astype(_F32)
        h_s[rows, :] = (_layernorm(xf) * (1.0 + mod_s[0:1, D:2 * D]) + mod_s[0:1, 0:D]).astype(_BF16)

    def store_windows(j, rows, kk):
        for g in range(NW):
            c0 = _win_start(g)
            kq_s[j, g, rows, :] = kk[:, c0:c0 + 128]

    def x_copy(r):
        rows = rows_of(r)
        return pltpu.make_async_copy(x_hbm.at[rows, :], x_v.at[rows, :], xsems.at[r])

    with jax.named_scope('prologue'):
        cp_ma.start()
        x_copy(0).start()
        cp_wk.start()
        cf = c_ref[...].astype(_F32)
        sc = jnp.broadcast_to(cf * jax.nn.sigmoid(cf), (8, D))

        cp_ma.wait()
        x_copy(1).start()
        x_copy(2).start()
        mod_s[...] = _dot(sc, wmoda_v[...])
        x_copy(0).wait()
        x_copy(3).start()
        cp_wq.start()
        cp_wv.start()
        ln1(0)
        cp_wk.wait()
        cp_mb.start()
        cp_wo.start()
        cp_wg.start()
        cp_wu.start()
        cp_wd.start()

        def kloop(r, _):
            @pl.when(r < NQ - 1)
            def _():
                x_copy(r + 1).wait()
            rn = jnp.minimum(r + 1, NQ - 1)
            for blk in range(TQ // RB):
                rows = pl.ds(pl.multiple_of(r * TQ + blk * RB, RB), RB)
                store_windows(0, rows, _dot(h_s[rows, :], wk_v[...]).astype(_BF16))
                ln1(rn, blk)
            return 0
        jax.lax.fori_loop(0, NQ, kloop, 0)

        cp_wq.wait()
        cp_wv.wait()
        cp_mb.wait()
        tail = jnp.where(jax.lax.broadcasted_iota(jnp.int32, (VR - DH, TQ), 0) == 0, 1.0, 0.0)

        def qvloop(r, _):
            rows = rows_of(r)
            hr = h_s[rows, :]
            store_windows(1, rows, (_dot(hr, wq_v[...]) * qscale).astype(_BF16))
            modb_s[r] = _dot(sc, wmodb_v[:, pl.ds(pl.multiple_of(r * D, 128), D)])
            vt = _dot(hr, wv_v[...]).T
            for h in range(H):
                vt_s[h, 0:DH, rows] = vt[DH * h:DH * (h + 1), :]
                vt_s[h, DH:VR, rows] = tail
            return 0
        jax.lax.fori_loop(0, NQ, qvloop, 0)

        g0, qm0 = get_qm(0, 0)
        mx = None
        for c in range(NC):
            mx = stage1_store(qk(g0, qm0, c), c, mx)
            if c == NA - 1:
                ma0 = jnp.max(mx, axis=0, keepdims=True)
        mb0 = jnp.max(mx, axis=0, keepdims=True)
        cp_wo.wait()
        cp_wg.wait()
        cp_wu.wait()
        cp_wd.wait()

    def out_copy(i):
        return pltpu.make_async_copy(
            o_v.at[i % 2], o_hbm.at[pl.ds(pl.multiple_of(i * TQ, TQ), TQ), :], osems.at[i % 2])

    def tile(i, ms):
        def unit(b, k, ms):
            ma, mb = ms
            h = b * UN + k
            hn = (h + 1) & (H - 1)
            qtn = jnp.minimum(i + ((h + 1) >> 5), NQ - 1)
            g, qm = get_qm(qtn, hn)
            mx = None
            acc = None
            for c in range(NC):
                if c == NA:
                    acc = acc * jnp.exp2(ma - mb)
                p = jnp.exp2(s1[c * CK:(c + 1) * CK, :] - (ma if c < NA else mb)).astype(_BF16)
                s = qk(g, qm, c)
                o = _dot(vt_s[h, :, c * CK:(c + 1) * CK], p)
                acc = o if acc is None else acc + o
                mx = stage1_store(s, c, mx)
                if c == NA - 1:
                    ma_n = jnp.max(mx, axis=0, keepdims=True)
            on = acc * (1.0 / acc[DH:DH + 1, :])
            ot_s[b, DH * k:DH * (k + 1), :] = on[0:DH, :]
            return ma_n, jnp.max(mx, axis=0, keepdims=True)

        def body(b, ms):
            for k in range(UN):
                ms = unit(b, k, ms)
            return ms

        @pl.when(i >= 2)
        def _():
            out_copy(i - 2).wait()

        with jax.named_scope('attn'):
            ms = jax.lax.fori_loop(0, H // UN, body, ms)

        ga, sb, cb, gb = [modb_s[k, 0:1, :] for k in range(4)]
        with jax.named_scope('post'):
            NSUB = 4
            HB = TQ // NSUB
            x1, h2 = [], []
            for a in range(NSUB):
                ot = ot_s[:, :, a * HB:(a + 1) * HB].reshape(D, HB)
                attn = _dot_tn(ot, wo_v[...])
                xt = x_v[pl.ds(pl.multiple_of(i * TQ + a * HB, HB), HB), :].astype(_F32)
                x1.append(xt + ga * attn)
                h2.append((_layernorm(x1[a]) * (1.0 + cb) + sb).astype(_BF16))
            acts = []
            for a in range(NSUB):
                gt = _dot_nt(h2[a], wg_v[0:FC, :])
                up = _dot_nt(h2[a], wu_v[0:FC, :])
                acts.append((_gelu_tanh(gt) * up).astype(_BF16))
            act = jnp.concatenate(acts, axis=0)
            h2 = jnp.concatenate(h2, axis=0)
            y = _dot(act, wd_v[0:FC, :])
            NF = F // FC
            for j in range(1, NF):
                f0, f1 = j * FC, (j + 1) * FC
                gt = _dot_nt(h2, wg_v[f0:f1, :])
                up = _dot_nt(h2, wu_v[f0:f1, :])
                act = (_gelu_tanh(gt) * up).astype(_BF16)
                y = y + _dot(act, wd_v[f0:f1, :])
            f0 = NF * FC
            gt = _dot_nt(h2, wg_v[f0:f0 + 128, :])
            up = _dot_nt(h2, wu_v[f0:f0 + 128, :])
            wr = jnp.concatenate([wg_v[f0 + 128:F, :], wu_v[f0 + 128:F, :]], axis=0)
            gu = _dot_nt(h2, wr)
            act = jnp.concatenate(
                [_gelu_tanh(gt) * up, _gelu_tanh(gu[:, 0:64]) * gu[:, 64:128]], axis=1).astype(_BF16)
            y = y + _dot(act, wd_v[f0:F, :])
            x1 = jnp.concatenate(x1, axis=0)

            o_v[i % 2] = (x1 + gb * y).astype(o_v.dtype)
            out_copy(i).start()
        return ms

    jax.lax.fori_loop(0, NQ, tile, (ma0, mb0))
    out_copy(NQ - 2).wait()
    out_copy(NQ - 1).wait()


@jax.jit
def pallas_adaLN_cond__mha_block__geglu_ffn__prompt_kernel(
    A_x, A_wqkv, A_wo, B_x, B_w_gate, B_w_up, B_w_down, c, w_mod,
):
    del B_x
    x2 = A_x.reshape(S, D)
    hbm = pl.BlockSpec(memory_space=pltpu.MemorySpace.HBM)
    out = pl.pallas_call(
        _kernel,
        in_specs=[pl.BlockSpec(memory_space=pltpu.MemorySpace.VMEM)] + [hbm] * 7,
        out_specs=hbm,
        out_shape=jax.ShapeDtypeStruct((S, D), A_x.dtype),
        scratch_shapes=[
            pltpu.VMEM((S, TQ), _F32),
            pltpu.VMEM((2, NW, S, 128), _BF16),
            pltpu.VMEM((H, VR, S), _F32),
            pltpu.VMEM((H // UN, UN * DH, TQ), _F32),
            pltpu.VMEM((S, D), _BF16),
            pltpu.VMEM((D, D), _BF16),
            pltpu.VMEM((D, D), _BF16),
            pltpu.VMEM((D, D), _BF16),
            pltpu.VMEM((D, D), _BF16),
            pltpu.VMEM((F, D), _BF16),
            pltpu.VMEM((F, D), _BF16),
            pltpu.VMEM((F, D), _BF16),
            pltpu.VMEM((D, 2 * D), _BF16),
            pltpu.VMEM((D, 4 * D), _BF16),
            pltpu.VMEM((8, 2 * D), _F32),
            pltpu.VMEM((4, 8, D), _F32),
            pltpu.VMEM((S, D), _BF16),
            pltpu.VMEM((2, TQ, D), _BF16),
            pltpu.SemaphoreType.DMA((9,)),
            pltpu.SemaphoreType.DMA((NQ,)),
            pltpu.SemaphoreType.DMA((2,)),
        ],
        compiler_params=pltpu.CompilerParams(
            vmem_limit_bytes=100 * 1024 * 1024,
        ),
    )(c, x2, A_wqkv, A_wo, B_w_gate.T, B_w_up.T, B_w_down, w_mod)
    return out.reshape(A_x.shape)
```

```python
import math

import jax
import jax.numpy as jnp
from jax.experimental import pallas as pl
from jax.experimental.pallas import tpu as pltpu

S = 2048
D = 640
H = 32
DH = 20
F = 1728
TQ = 512
NQ = S // TQ
CK = 128
NC = S // CK
NA = 12
UN = 8
NW = 6
VR = 24
NSUB = 4
FC = 256
EPS = 1e-5

_NT = (((1,), (1,)), ((), ()))
_TN = (((0,), (0,)), ((), ()))
_F32 = jnp.float32
_BF16 = jnp.bfloat16


def _win_start(g):
    return 120 * g if g < NW - 1 else D - 128


def _layernorm(xf):
    m = jnp.mean(xf, axis=-1, keepdims=True)
    xc = xf - m
    v = jnp.mean(xc * xc, axis=-1, keepdims=True)
    return xc * jax.lax.rsqrt(v + EPS)


def _gelu_tanh(x):
    c = math.sqrt(2.0 / math.pi)
    return 0.5 * x * (1.0 + jnp.tanh(c * (x + 0.044715 * (x * x * x))))


def _dot(a, b):
    return jnp.dot(a, b, preferred_element_type=_F32)


def _dot_nt(a, b):
    return jax.lax.dot_general(a, b, _NT, preferred_element_type=_F32)


def _dot_tn(a, b):
    return jax.lax.dot_general(a, b, _TN, preferred_element_type=_F32)


def _kernel(c_ref, x_hbm, wqkv_hbm, wo_hbm, wg_hbm, wu_hbm, wd_hbm, wmod_hbm,
            o_hbm,
            s1, kq_s, vt_s, ot_s,
            x_v, wq_v, wk_v, wv_v, wo_v, wg_v, wu_v, wd_v, wmoda_v, wmodb_v,
            mod_s, modb_s, h_s, o_v,
            sems, xsems, osems):
    cp_wk = pltpu.make_async_copy(wqkv_hbm.at[:, D:2 * D], wk_v, sems.at[0])
    cp_ma = pltpu.make_async_copy(wmod_hbm.at[:, 0:2 * D], wmoda_v, sems.at[1])
    cp_wq = pltpu.make_async_copy(wqkv_hbm.at[:, 0:D], wq_v, sems.at[2])
    cp_wv = pltpu.make_async_copy(wqkv_hbm.at[:, 2 * D:3 * D], wv_v, sems.at[3])
    cp_wo = pltpu.make_async_copy(wo_hbm, wo_v, sems.at[4])
    cp_mb = pltpu.make_async_copy(wmod_hbm.at[:, 2 * D:6 * D], wmodb_v, sems.at[5])
    cp_wg = pltpu.make_async_copy(wg_hbm, wg_v, sems.at[6])
    cp_wu = pltpu.make_async_copy(wu_hbm, wu_v, sems.at[7])
    cp_wd = pltpu.make_async_copy(wd_hbm, wd_v, sems.at[8])

    def rows_of(r):
        if isinstance(r, int):
            return slice(r * TQ, (r + 1) * TQ)
        return pl.ds(pl.multiple_of(r * TQ, TQ), TQ)

    def x_copy(r):
        rows = rows_of(r)
        return pltpu.make_async_copy(x_hbm.at[rows, :], x_v.at[rows, :], xsems.at[r])

    def out_copy(i):
        return pltpu.make_async_copy(o_v.at[i % 2], o_hbm.at[rows_of(i), :], osems.at[i % 2])

    lane = jax.lax.broadcasted_iota(jnp.int32, (TQ, 128), 1)

    def get_qm(qt, h):
        g = (h * 43) >> 8
        off = DH * h - 120 * g + jnp.where(g == NW - 1, 120 * (NW - 1) - (D - 128), 0)
        qw = kq_s[1, g, rows_of(qt), :]
        mask = (lane >= off) & (lane < off + DH)
        return g, jnp.where(mask, qw, jnp.zeros_like(qw))

    def scores(g, qm, c):
        return _dot_nt(kq_s[0, g, c * CK:(c + 1) * CK, :], qm)

    def store_scores(s, c, mx):
        s1[c * CK:(c + 1) * CK, :] = s
        cm = jnp.max(s.reshape(CK // 8, 8, TQ), axis=0)
        return cm if mx is None else jnp.maximum(mx, cm)

    def ln1(rows):
        xf = x_v[rows, :].astype(_F32)
        h_s[rows, :] = (_layernorm(xf) * (1.0 + mod_s[0:1, D:2 * D]) + mod_s[0:1, 0:D]).astype(_BF16)

    def store_windows(j, rows, kk):
        for g in range(NW):
            c0 = _win_start(g)
            kq_s[j, g, rows, :] = kk[:, c0:c0 + 128]

    cp_ma.start()
    x_copy(0).start()
    cp_wk.start()
    cf = c_ref[...].astype(_F32)
    sc = jnp.broadcast_to(cf * jax.nn.sigmoid(cf), (8, D))

    cp_ma.wait()
    mod_s[...] = _dot(sc, wmoda_v[...])
    x_copy(0).wait()
    x_copy(1).start()
    x_copy(2).start()
    x_copy(3).start()
    cp_wq.start()
    cp_wv.start()
    ln1(rows_of(0))
    cp_wk.wait()
    cp_mb.start()
    cp_wo.start()
    cp_wg.start()
    cp_wu.start()
    cp_wd.start()

    def kloop(r, carry):
        rows = rows_of(r)
        hr = h_s[rows, :]
        kk = [_dot(hr, wk_v[:, 128 * n:128 * (n + 1)]).astype(_BF16) for n in range(D // 128)]
        store_windows(0, rows, jnp.concatenate(kk, axis=1))

        @pl.when(r < NQ - 1)
        def _():
            x_copy(r + 1).wait()
            ln1(rows_of(r + 1))
        return carry
    jax.lax.fori_loop(0, NQ, kloop, 0)

    cp_wq.wait()
    cp_wv.wait()
    cp_mb.wait()
    qscale = (DH ** -0.5) * math.log2(math.e)
    tail = jnp.where(jax.lax.broadcasted_iota(jnp.int32, (VR - DH, TQ), 0) == 0, 1.0, 0.0)

    def qvloop(r, carry):
        rows = rows_of(r)
        hr = h_s[rows, :]
        vt = _dot(hr, wv_v[...]).T
        for h in range(H):
            vt_s[h, 0:DH, rows] = vt[DH * h:DH * (h + 1), :]
            vt_s[h, DH:VR, rows] = tail
        modb_s[r] = _dot(sc, wmodb_v[:, pl.ds(pl.multiple_of(r * D, 128), D)])
        store_windows(1, rows, (_dot(hr, wq_v[...]) * qscale).astype(_BF16))
        return carry
    jax.lax.fori_loop(0, NQ, qvloop, 0)

    g0, qm0 = get_qm(0, 0)
    mx = None
    for c in range(NC):
        mx = store_scores(scores(g0, qm0, c), c, mx)
        if c == NA - 1:
            ma0 = jnp.max(mx, axis=0, keepdims=True)
    mb0 = jnp.max(mx, axis=0, keepdims=True)
    cp_wo.wait()
    cp_wg.wait()
    cp_wu.wait()
    cp_wd.wait()

    def tile(i, ms):
        def unit(b, k, ms):
            ma, mb = ms
            h = b * UN + k
            hn = (h + 1) & (H - 1)
            qtn = jnp.minimum(i + ((h + 1) >> 5), NQ - 1)
            g, qm = get_qm(qtn, hn)
            mx = None
            acc = None
            for c in range(NC):
                if c == NA:
                    acc = acc * jnp.exp2(ma - mb)
                p = jnp.exp2(s1[c * CK:(c + 1) * CK, :] - (ma if c < NA else mb)).astype(_BF16)
                o = _dot(vt_s[h, :, c * CK:(c + 1) * CK], p)
                s = scores(g, qm, c)
                acc = o if acc is None else acc + o
                mx = store_scores(s, c, mx)
                if c == NA - 1:
                    ma_n = jnp.max(mx, axis=0, keepdims=True)
            on = acc * (1.0 / acc[DH:DH + 1, :])
            ot_s[b, DH * k:DH * (k + 1), :] = on[0:DH, :]
            return ma_n, jnp.max(mx, axis=0, keepdims=True)

        def body(b, ms):
            for k in range(UN):
                ms = unit(b, k, ms)
            return ms

        @pl.when(i >= 2)
        def _():
            out_copy(i - 2).wait()

        ms = jax.lax.fori_loop(0, H // UN, body, ms)

        ga, sb, cb, gb = [modb_s[k, 0:1, :] for k in range(4)]
        hb = TQ // NSUB
        x1, h2 = [], []
        for a in range(NSUB):
            ot = ot_s[:, :, a * hb:(a + 1) * hb].reshape(D, hb)
            attn = _dot_tn(ot, wo_v[...])
            xt = x_v[pl.ds(pl.multiple_of(i * TQ + a * hb, hb), hb), :].astype(_F32)
            x1.append(xt + ga * attn)
            h2.append((_layernorm(x1[a]) * (1.0 + cb) + sb).astype(_BF16))
        acts = []
        for a in range(NSUB):
            gt = _dot_nt(h2[a], wg_v[0:FC, :])
            up = _dot_nt(h2[a], wu_v[0:FC, :])
            acts.append((_gelu_tanh(gt) * up).astype(_BF16))
        act = jnp.concatenate(acts, axis=0)
        h2 = jnp.concatenate(h2, axis=0)
        y = _dot(act, wd_v[0:FC, :])
        nf = F // FC
        for j in range(1, nf):
            f0, f1 = j * FC, (j + 1) * FC
            gt = _dot_nt(h2, wg_v[f0:f1, :])
            up = _dot_nt(h2, wu_v[f0:f1, :])
            act = (_gelu_tanh(gt) * up).astype(_BF16)
            y = y + _dot(act, wd_v[f0:f1, :])
        f0 = nf * FC
        gt = _dot_nt(h2, wg_v[f0:f0 + 128, :])
        up = _dot_nt(h2, wu_v[f0:f0 + 128, :])
        wr = jnp.concatenate([wg_v[f0 + 128:F, :], wu_v[f0 + 128:F, :]], axis=0)
        gu = _dot_nt(h2, wr)
        act = jnp.concatenate(
            [_gelu_tanh(gt) * up, _gelu_tanh(gu[:, 0:64]) * gu[:, 64:128]], axis=1).astype(_BF16)
        y = y + _dot(act, wd_v[f0:F, :])
        x1 = jnp.concatenate(x1, axis=0)
        o_v[i % 2] = (x1 + gb * y).astype(o_v.dtype)
        out_copy(i).start()
        return ms

    jax.lax.fori_loop(0, NQ, tile, (ma0, mb0))
    out_copy(NQ - 2).wait()
    out_copy(NQ - 1).wait()


@jax.jit
def pallas_adaLN_cond__mha_block__geglu_ffn__prompt_kernel(
    A_x, A_wqkv, A_wo, B_x, B_w_gate, B_w_up, B_w_down, c, w_mod,
):
    del B_x
    x2 = A_x.reshape(S, D)
    hbm = pl.BlockSpec(memory_space=pltpu.MemorySpace.HBM)
    out = pl.pallas_call(
        _kernel,
        in_specs=[pl.BlockSpec(memory_space=pltpu.MemorySpace.VMEM)] + [hbm] * 7,
        out_specs=hbm,
        out_shape=jax.ShapeDtypeStruct((S, D), A_x.dtype),
        scratch_shapes=[
            pltpu.VMEM((S, TQ), _F32),
            pltpu.VMEM((2, NW, S, 128), _BF16),
            pltpu.VMEM((H, VR, S), _F32),
            pltpu.VMEM((H // UN, UN * DH, TQ), _F32),
            pltpu.VMEM((S, D), _BF16),
            pltpu.VMEM((D, D), _BF16),
            pltpu.VMEM((D, D), _BF16),
            pltpu.VMEM((D, D), _BF16),
            pltpu.VMEM((D, D), _BF16),
            pltpu.VMEM((F, D), _BF16),
            pltpu.VMEM((F, D), _BF16),
            pltpu.VMEM((F, D), _BF16),
            pltpu.VMEM((D, 2 * D), _BF16),
            pltpu.VMEM((D, 4 * D), _BF16),
            pltpu.VMEM((8, 2 * D), _F32),
            pltpu.VMEM((4, 8, D), _F32),
            pltpu.VMEM((S, D), _BF16),
            pltpu.VMEM((2, TQ, D), _BF16),
            pltpu.SemaphoreType.DMA((9,)),
            pltpu.SemaphoreType.DMA((NQ,)),
            pltpu.SemaphoreType.DMA((2,)),
        ],
        compiler_params=pltpu.CompilerParams(
            vmem_limit_bytes=100 * 1024 * 1024,
        ),
    )(c, x2, A_wqkv, A_wo, B_w_gate.T, B_w_up.T, B_w_down, w_mod)
    return out.reshape(A_x.shape)
```
